```python
import os as _os
_os.environ.setdefault("JAX_PLATFORMS", "cpu")
import jax
import jax.numpy as jnp

def _softmax(x, axis=-1):
    return jax.nn.softmax(x, axis=axis)
def _gelu(x):
    return jax.nn.gelu(x, approximate=True)
def _silu(x):
    return jax.nn.silu(x)
def _sigmoid(x):
    return jax.nn.sigmoid(x)
def _layernorm(x, axis=-1, eps=1e-5):
    m = jnp.mean(x, axis=axis, keepdims=True)
    v = jnp.var(x, axis=axis, keepdims=True)
    return (x - m) / jnp.sqrt(v + eps)
def _scatter_add(tgt, idx, src, axis=0):
    return tgt.at[idx].add(src)
def _segment_sum(src, seg, n):
    return jax.ops.segment_sum(src, seg, n)
class _Rng:
    def __init__(self, key):
        self._k = key
    def _next(self):
        self._k, sub = jax.random.split(self._k)
        return sub
    def normal(self, shape):
        return jax.random.normal(self._next(), shape, dtype=jnp.bfloat16)
    def randint(self, lo, hi, shape):
        return jax.random.randint(self._next(), shape, lo, hi, dtype=jnp.int32)
    def uniform(self, shape, lo=0.0, hi=1.0):
        return jax.random.uniform(self._next(), shape, jnp.bfloat16, lo, hi)
    def permutation(self, n):
        return jax.random.permutation(self._next(), n)


kernel_name = 'concat_heads__mha_block_cached__gqa_block_cached__near_ridge'

def setup_inputs():
    _rng = _Rng(jax.random.key(int.from_bytes(__import__("os").urandom(4), "little")))
    _w = (lambda a: (lambda t: t.astype(jnp.bfloat16) if jnp.issubdtype(t.dtype, jnp.floating) else t)(jnp.asarray(a)))
    def _A_setup():
        B, Sq, D = 16, 160, 512
        H, Sk, Dh = 32, 1024, 128
        return {
            "x": _w((lambda *s: _rng.normal(s) * 0.8)(B, Sq, D)),
            "k_cache": _w((lambda *s: _rng.normal(s) * 0.8)(B, H, Sk, Dh)),
            "v_cache": _w((lambda *s: _rng.normal(s) * 0.05)(B, H, Sk, Dh)),
            "wq": _w((lambda *s: _rng.normal(s) * 0.8)(D, H * Dh) * (D ** -0.5)),
            "wo": _w((lambda *s: _rng.normal(s) * 0.05)(H * Dh, D) * ((H * Dh) ** -0.5)),
        }
    _A_in = _A_setup()

    def _B_setup():
        B, Sq, D = 16, 160, 512
        Hq, Hkv, Sk, Dh = 32, 32, 1024, 128
        assert Hq % Hkv == 0, (Hq, Hkv)
        return {
            "x": _w((lambda *s: _rng.normal(s) * 0.8)(B, Sq, D)),
            "k_cache": _w((lambda *s: _rng.normal(s) * 0.8)(B, Hkv, Sk, Dh)),
            "v_cache": _w((lambda *s: _rng.normal(s) * 0.05)(B, Hkv, Sk, Dh)),
            "wq": _w((lambda *s: _rng.normal(s) * 0.8)(D, Hq * Dh) * (D ** -0.5)),
            "wo": _w((lambda *s: _rng.normal(s) * 0.05)(Hq * Dh, D) * ((Hq * Dh) ** -0.5)),
        }
    _B_in = _B_setup()

    return {
        "A_x": _A_in["x"],
        "A_k_cache": _A_in["k_cache"],
        "A_v_cache": _A_in["v_cache"],
        "A_wq": _A_in["wq"],
        "A_wo": _A_in["wo"],
        "B_x": _B_in["x"],
        "B_k_cache": _B_in["k_cache"],
        "B_v_cache": _B_in["v_cache"],
        "B_wq": _B_in["wq"],
        "B_wo": _B_in["wo"],
    }

def reference(A_x, A_k_cache, A_v_cache, A_wq, A_wo, B_x, B_k_cache, B_v_cache, B_wq, B_wo):
    def _A_ref(x, k_cache, v_cache, wq, wo):
        B, Sq, D = x.shape
        H, Dh = 32, 128
        q = (lambda x, *d: x.transpose(*d))((x @ wq).reshape(B, Sq, H, Dh), 0, 2, 1, 3)
        scores = jnp.einsum("bhqd,bhkd->bhqk", q, k_cache) * (Dh ** -0.5)
        p = _softmax(scores, axis=-1)
        o = jnp.einsum("bhqk,bhkd->bhqd", p, v_cache)
        return (lambda x, *d: x.transpose(*d))(o, 0, 2, 1, 3).reshape(B, Sq, H * Dh) @ wo

    def _B_ref(x, k_cache, v_cache, wq, wo):
        B, Sq, D = x.shape
        Hq, Dh = 32, 128
        Hkv = k_cache.shape[1]
        rep = Hq // Hkv
        q = (lambda x, *d: x.transpose(*d))((x @ wq).reshape(B, Sq, Hq, Dh), 0, 2, 1, 3)
        k = jnp.repeat(k_cache, rep, axis=1)
        v = jnp.repeat(v_cache, rep, axis=1)
        scores = jnp.einsum("bhqd,bhkd->bhqk", q, k) * (Dh ** -0.5)
        p = _softmax(scores, axis=-1)
        o = jnp.einsum("bhqk,bhkd->bhqd", p, v)
        return (lambda x, *d: x.transpose(*d))(o, 0, 2, 1, 3).reshape(B, Sq, Hq * Dh) @ wo

    a = _A_ref(A_x, A_k_cache, A_v_cache, A_wq, A_wo)
    b = _B_ref(B_x, B_k_cache, B_v_cache, B_wq, B_wo)
    return jnp.concatenate([a, b], axis=-1)
```

```python
import functools, math
import jax, jax.numpy as jnp, numpy as np
from jax import lax
from jax.experimental import pallas as pl
from jax.experimental.pallas import tpu as pltpu

B, Sq, D, H, Sk, Dh = 16, 160, 512, 32, 1024, 128
QSCALE = float(Dh ** -0.5 * math.log2(math.e))
f32, bf16 = jnp.float32, jnp.bfloat16

def make(G=4, NG=4, nodma=False, prio=(0, 0), order=None, rb=160, nobc=True, newton=True, wb_at=None, oprio=0, wprio=0):
    if order is None:
        order = "s0 o " + " ".join(f"s{h + 1} p{h}" for h in range(G - 1)) + f" q p{G - 1}"
    GB = H // G
    NH = B * GB
    N = 2 * NH
    W = G * Dh
    LG = GB.bit_length() - 1
    LH = NH.bit_length() - 1
    wb_at = NH // 2 if wb_at is None else wb_at

    def split(i):
        return i >> LH, (i >> LG) & (B - 1), i & (GB - 1)

    def kern(ax, ak, av, awq, awo, bx, bk, bv, bwq, bwo, o_hbm,
             kbuf, vbuf, wq_s, wo_s, x_s, q_s, o_s, acc, out_s, ksem, vsem, wsem, osem):
        def kv_copy(src, buf, sem, i, slot):
            _, b, g = split(i)
            return pltpu.make_async_copy(src.at[b, pl.ds(g * G, G)], buf.at[slot], sem.at[slot])

        def start_group(ksrc, vsrc, i, slot):
            kv_copy(ksrc, kbuf, ksem, i, slot).start(priority=prio[0])
            kv_copy(vsrc, vbuf, vsem, i, slot).start(priority=prio[1])

        wa = [pltpu.make_async_copy(ax, x_s.at[0], wsem.at[0]),
              pltpu.make_async_copy(awq, wq_s.at[0], wsem.at[1]),
              pltpu.make_async_copy(awo, wo_s.at[0], wsem.at[2])]
        wb = [pltpu.make_async_copy(bx, x_s.at[1], wsem.at[3]),
              pltpu.make_async_copy(bwq, wq_s.at[1], wsem.at[4]),
              pltpu.make_async_copy(bwo, wo_s.at[1], wsem.at[5])]
        for c in wa:
            c.start(priority=wprio)
        for s in range(NG - 1):
            start_group(ak, av, s, s)
        if nodma:
            start_group(ak, av, NG - 1, NG - 1)
            for s in range(NG):
                kv_copy(ak, kbuf, ksem, s, s).wait()
                kv_copy(av, vbuf, vsem, s, s).wait()

        def qproj(i):
            half, b, g = split(i)
            col = pl.multiple_of(g * W, W)
            q = jnp.dot(x_s[half, b], wq_s[half, :, pl.ds(col, W)], preferred_element_type=f32)
            for h in range(G):
                q_s[h] = (q[:, h * Dh:(h + 1) * Dh] * QSCALE).astype(bf16)

        def oproj(i):
            half, b, g = split(i)
            row = pl.multiple_of(g * W, W)
            o = jnp.concatenate([o_s[h] for h in range(G)], axis=-1)
            r = jnp.dot(o, wo_s[half, pl.ds(row, W), :], preferred_element_type=f32)
            r = r + jnp.where(g == 0, 0.0, acc[...])
            acc[...] = r
            out_s[b, :, pl.ds(pl.multiple_of(half * D, D), D)] = r.astype(bf16)

        o_s[...] = jnp.zeros_like(o_s)
        acc[...] = jnp.zeros_like(acc)
        wa[0].wait(); wa[1].wait()
        qproj(0)
        wa[2].wait()
        out_head = pltpu.make_async_copy(out_s.at[pl.ds(0, B - 1)], o_hbm.at[pl.ds(0, B - 1)], osem.at[0])
        out_tail = pltpu.make_async_copy(out_s.at[B - 1], o_hbm.at[B - 1], osem.at[1])

        def body(i, slot):
            nxt = i + NG - 1
            nslot = jnp.where(slot == 0, NG - 1, slot - 1)
            if not nodma:
                @pl.when(nxt < NH)
                def _():
                    start_group(ak, av, nxt, nslot)
                @pl.when(jnp.logical_and(nxt >= NH, nxt < N))
                def _():
                    start_group(bk, bv, nxt, nslot)
            @pl.when(i == wb_at)
            def _():
                for c in wb:
                    c.start(priority=wprio)
            @pl.when(i == NH - 1)
            def _():
                for c in wb:
                    c.wait()
            @pl.when(i == max(N - NG + 1, N - GB + 1))
            def _():
                out_head.start(priority=oprio)
            if not nodma:
                kv_copy(ak, kbuf, ksem, i, slot).wait()
                kv_copy(av, vbuf, vsem, i, slot).wait()

            def qk(h):
                s = lax.dot_general(q_s[h], kbuf[slot, h], (((1,), (1,)), ((), ())), preferred_element_type=f32)
                ps, ls = [], []
                for r in range(0, Sq, rb):
                    sr = s[r:r + rb]
                    m = jnp.max(sr, axis=-1, keepdims=True)
                    p = jnp.exp2(sr - m)
                    ls.append(jnp.sum(p, axis=-1, keepdims=True))
                    ps.append(p.astype(bf16))
                return jnp.concatenate(ps, axis=0), jnp.concatenate(ls, axis=0)
            def pv(h, p, l):
                o = jnp.dot(p, vbuf[slot, h], preferred_element_type=f32)
                if newton:
                    r = pl.reciprocal(l, approx=True)
                    r = r * (2.0 - l * r)
                else:
                    r = pl.reciprocal(l)
                o_s[h] = (o * r).astype(bf16)
            pend = {}
            for op in order.split():
                if op == "o":
                    oproj(jnp.maximum(i - 1, 0))
                elif op == "q":
                    qproj(jnp.minimum(i + 1, N - 1))
                elif op[0] == "s":
                    pend[int(op[1:])] = qk(int(op[1:]))
                elif op[0] == "p":
                    pv(int(op[1:]), *pend.pop(int(op[1:])))
            return jnp.where(slot == NG - 1, 0, slot + 1)
        lax.fori_loop(0, N, body, jnp.int32(0))
        oproj(N - 1)
        out_tail.start()
        out_head.wait()
        out_tail.wait()

    def kernel_v4(*a):
        return pl.pallas_call(
            kern,
            in_specs=[pl.BlockSpec(memory_space=pl.ANY)] * 10,
            out_specs=pl.BlockSpec(memory_space=pl.ANY),
            out_shape=jax.ShapeDtypeStruct((B, Sq, 2 * D), bf16),
            scratch_shapes=[
                pltpu.VMEM((NG, G, Sk, Dh), bf16), pltpu.VMEM((NG, G, Sk, Dh), bf16),
                pltpu.VMEM((2, D, H * Dh), bf16), pltpu.VMEM((2, H * Dh, D), bf16),
                pltpu.VMEM((2, B, Sq, D), bf16),
                pltpu.VMEM((G, Sq, Dh), bf16), pltpu.VMEM((G, Sq, Dh), bf16),
                pltpu.VMEM((Sq, D), f32), pltpu.VMEM((B, Sq, 2 * D), bf16),
                pltpu.SemaphoreType.DMA((NG,)), pltpu.SemaphoreType.DMA((NG,)),
                pltpu.SemaphoreType.DMA((6,)), pltpu.SemaphoreType.DMA((2,))],
            compiler_params=pltpu.CompilerParams(vmem_limit_bytes=120 * 2**20, disable_bounds_checks=nobc),
        )(*a)
    return kernel_v4


@jax.jit
def pallas_concat_heads__mha_block_cached__gqa_block_cached__near_ridge_kernel(
        A_x, A_k_cache, A_v_cache, A_wq, A_wo, B_x, B_k_cache, B_v_cache, B_wq, B_wo):
    return make(G=4, NG=4)(A_x, A_k_cache, A_v_cache, A_wq, A_wo, B_x, B_k_cache, B_v_cache, B_wq, B_wo)
```

```python
import functools, math
import jax, jax.numpy as jnp, numpy as np
from jax import lax
from jax.experimental import pallas as pl
from jax.experimental.pallas import tpu as pltpu

B, Sq, D, H, Sk, Dh = 16, 160, 512, 32, 1024, 128
QSCALE = float(Dh ** -0.5 * math.log2(math.e))
f32, bf16, u32 = jnp.float32, jnp.bfloat16, jnp.uint32
NT = (((1,), (1,)), ((), ()))
G = 8
N = 128
NG = 3
CR = 128
NC = Sk // CR
KV = 2 * G * Sk

def lin(basis):
    o = [0]
    for v in basis:
        o = o + [x ^ v for x in o]
    return o

SCHED = "QSSQPP SSQPP SSQPP SSQPP SSOQPP OSSQPP SSOPP SSOPPQ OOOO"

def make(hbits=(2, 3, 4), sched=SCHED, basis=(8, 16, 32, 1, 2, 4), arr=(0,) * 64 + (1,) * 64, pri=("110", "110", "10"),
         rot=64, table=False, flags=None, order=None, wpri="110", spri="110", newton=True, nosemchk=True, scope=False,
         wrate=3, wstride=17, qstride=17, ballast=False, xt=(5, 11, 20, 32, 44), sm="c", ukv=True, skip0=False, odl=2, olast=0, qpad=128, carry=True):
    gbits = [t for t in range(5) if t not in hbits]
    hoff = [sum(((j >> t) & 1) << hbits[t] for t in range(3)) for j in range(G)]
    def gbase(g):
        return ((g & 1) << gbits[0]) | (((g >> 1) & 1) << gbits[1])
    def head(ph, j):
        hh = gbase(ph)
        for e in range(3):
            hh = hh + (((j >> e) & 1) << hbits[e])
        return hh
    order = order or (lin(basis), lin(basis))
    names = sched.replace(" ", "")
    NP = len(names)
    assert [names.count(c) for c in "QSPO"] == [8, 16, 16, 8]
    seq, cnt = [], [0, 0]
    for c in range(2 * G * NC):
        a = arr[c % len(arr)]
        seq.append((a, cnt[a])); cnt[a] += 1
    assert cnt == [G * NC, G * NC], cnt
    points, c = [], rot
    for t in range(NP):
        lst = []
        for ch in pri[t % len(pri)]:
            lst.append((1 + c // len(seq),) + seq[c % len(seq)] + (int(ch),))
            c += 1
        points.append(lst)
    assert c == rot + len(seq)
    if skip0:
        points[1] = points[0] + points[1]; points[0] = []
    sp = [int(c) for c in spri]
    wr = {}
    slots = [(N - 2, t) for t in range(NP) if points[t] and all(e[0] == 2 for e in points[t])] + [(N - 1, t) for t in range(NP) if points[t]]
    first = [(w * wstride) % 140 for w in range(140)]
    assert sorted(first) == list(range(140))
    todo = [divmod(w, 10) for w in first + list(range(140, 150))]
    w = 0
    for k, s in enumerate(slots):
        while todo and s[0] > N - B + todo[0][0] and (w < wrate * (k + 1) or s == slots[-1]):
            wr.setdefault(s, []).append(todo.pop(0) + (int(wpri[w % len(wpri)]),)); w += 1
    assert not todo

    def kern(*refs):
        if table:
            tab, *refs = refs
        (ax, ak, av, awq, awo, bx, bk, bv, bwq, bwo, o_hbm,
         buf, wq_s, wo_s, x_s, q_s, acc, out_s, sem) = refs
        QS, OS, XS, WS = NG, NG + 2, NG + 4, NG + 8

        def tile(r):
            return buf.at[pl.ds(pl.multiple_of(r, CR), CR)]
        def kv_start(srcs, i, slot, lst):
            base = ((i & 15) * H + gbase(i >> 4)) * Sk
            for a, n, pr in lst:
                if table:
                    src = base + tab[(a * 64 + n) * 2]
                    dst = tab[(a * 64 + n) * 2 + 1]
                else:
                    j, c = divmod(order[a][n], NC)
                    src = base + hoff[j] * Sk + c * CR
                    dst = j * Sk + c * CR
                pltpu.make_async_copy(srcs[a].at[pl.ds(pl.multiple_of(src, CR), CR)], tile(slot * KV + a * G * Sk + dst), sem.at[slot]).start(priority=pr)
        def wq_piece(src, half, t):
            t = (t * qstride) & 127
            r = pl.ds(pl.multiple_of((t >> 1) * 8, 8), 8)
            c = pl.ds(pl.multiple_of((t & 1) * 2048, 2048), 2048)
            return pltpu.make_async_copy(src.at[r, c], wq_s.at[half, r, c], sem.at[QS + half])
        def wo_piece(src, ph, t):
            j, r = t & 7, (t >> 3) * 32
            return pltpu.make_async_copy(src.at[pl.ds(pl.multiple_of(head(ph, j) * Dh + r, 32), 32)],
                                         wo_s.at[ph, pl.ds(pl.multiple_of(j * Dh + r, 32), 32)], sem.at[OS + (ph & 1)])
        def x_piece(src, half, b, u):
            return pltpu.make_async_copy(src.at[b, pl.ds(u * 32, 32)], x_s.at[half * B + b, pl.ds(u * 32, 32)], sem.at[XS + (b & 3)])
        def out_piece(b, u):
            return pltpu.make_async_copy(out_s.at[b, pl.ds(u * 16, 16)], o_hbm.at[b, pl.ds(u * 16, 16)], sem.at[WS])
        def full_wait(ref, s):
            pltpu.make_async_copy(ref, ref, sem.at[s]).wait()
        def ldw(r):
            if ukv:
                return pltpu.bitcast(buf.bitcast(u32)[pl.ds(pl.multiple_of(r >> 1, 256), 256), :], bf16)
            return buf[pl.ds(pl.multiple_of(r, 512), 512), :]

        @pl.loop(0, 32)
        def _(t):
            cps = []
            for e in range(2):
                n = 2 * t + e
                src = pl.multiple_of(head(0, n & 7) * Sk + (n >> 3) * CR, CR)
                dst = (n & 7) * Sk + (n >> 3) * CR
                for a, ref in enumerate((ak, av)):
                    cps.append(pltpu.make_async_copy(ref.at[pl.ds(src, CR)], tile(a * G * Sk + dst), sem.at[0]))
                    cps.append(wq_piece(awq, 0, 2 * n + a))
            cps.append(wo_piece(awo, 0, t))
            for c, cp in enumerate(cps):
                cp.start(priority=sp[c % len(sp)])
        @pl.loop(0, 3)
        def _(b):
            for u in range(5):
                x_piece(ax, 0, b, u).start(priority=u % 2)
        @pl.loop(0, 4)
        def _(t):
            wq_piece(bwq, 1, 2 * t).start(priority=1)
            wo_piece(awo, 1, t).start(priority=1)
            wq_piece(bwq, 1, 2 * t + 1).start(priority=0)
        kv_start((ak, av), 1, 1, [e + (sp[c % len(sp)],) for c, e in enumerate(seq[:rot])])
        full_wait(x_s.at[0], XS)
        wq_all = lambda half: wq_s.at[half, :, pl.ds(0, H * Dh)]
        full_wait(wq_all(0), QS)
        def arrive(i, slot):
            @pl.when(jnp.logical_and((i & 15) == 0, i < N))
            def _():
                full_wait(wo_s.at[i >> 4], OS + ((i >> 4) & 1))
            @pl.when(i == 63)
            def _():
                full_wait(wq_all(1), QS + 1)
            @pl.when(jnp.logical_and(((i + 1) & 63) < 16, i < N - 1))
            def _():
                full_wait(x_s.at[((i + 1) >> 6) * B + ((i + 1) & 15)], XS + ((i + 1) & 3))
            def kvw():
                @pl.when(i < N)
                def _():
                    full_wait(buf.at[pl.ds(pl.multiple_of(slot * KV, KV), KV)], slot)
            if scope:
                with jax.named_scope('kvwait'):
                    kvw()
            else:
                kvw()

        def wq_tile(j, h):
            return wq_s[j >> 6, :, pl.ds(pl.multiple_of((gbase(j >> 4) + hoff[h]) * Dh, Dh), Dh)]
        q_s[0] = (jnp.dot(x_s[0], wq_tile(0, 0), preferred_element_type=f32) * QSCALE).astype(bf16)

        arrive(jnp.int32(0), 0)
        def body(i, slot):
            slot1 = jnp.where(slot == NG - 1, 0, slot + 1)
            slot2 = jnp.where(slot == 0, NG - 1, slot - 1)
            b, ph = i & 15, i >> 4
            def both(e, fa, fb):
                pl.when(e < 64)(fa)
                pl.when(jnp.logical_and(e >= 64, e < N))(fb)
            def issue(t):
                k = names[:t].count(names[t])
                if names[t] == "O":
                    e = jnp.where((i & 3) == (k & 3), i + 18, N)
                    u = (e & 15) * 2 + k // 4
                    both(e, lambda: wo_piece(awo, e >> 4, u).start(priority=1), lambda: wo_piece(bwo, e >> 4, u).start(priority=1))
                if names[t] == "Q":
                    @pl.when(jnp.logical_and(((i + 2) & 3) == (k & 3), i + 4 < 64))
                    def _():
                        wq_piece(bwq, 1, (i + 4) * 2 + k // 4).start(priority=1)
                for d, sl in ((1, slot1), (2, slot2)):
                    lst = [e[1:] for e in points[t] if e[0] == d]
                    if lst:
                        both(i + d, lambda: kv_start((ak, av), i + d, sl, lst), lambda: kv_start((bk, bv), i + d, sl, lst))
                if ballast and t in (8, 23, 35, 47):
                    @pl.when(jnp.logical_and(i >= 80, i < N - 2))
                    def _():
                        wq_piece(awq, 0, i * 4 + (8, 23, 35, 47).index(t)).start(priority=1)
                if t in xt:
                    u = xt.index(t)
                    @pl.when(i + 3 < 16)
                    def _():
                        x_piece(ax, 0, i + 3, u).start(priority=1)
                    @pl.when(jnp.logical_and(i + 3 >= 64, i + 3 < 80))
                    def _():
                        x_piece(bx, 1, i + 3 - 64, u).start(priority=1)
                for it in (N - 2, N - 1):
                    if (it, t) in wr:
                        @pl.when(i == it)
                        def _():
                            for bb, u, pr in wr[it, t]:
                                out_piece(bb, u).start(priority=pr)

            st = {}
            nn = lambda a, w: jnp.dot(a, w, preferred_element_type=f32)
            def fold(t, op):
                return op(op(t[:, :128], t[:, 128:256]), op(t[:, 256:384], t[:, 384:]))
            def Q(k):
                j, h = (i, k + 1) if k < G - 1 else (jnp.minimum(i + 1, N - 1), 0)
                def fin(q):
                    q_s[h] = (q * QSCALE).astype(bf16)
                return lambda: wq_tile(j, h), lambda: x_s[(j >> 6) * B + (j & 15)], nn, fin
            def S(k):
                h, u = divmod(k, 2)
                def fin(s):
                    st["s", h, u] = s
                    if u == 1:
                        s0 = st["s", h, 0]
                        if sm == "a":
                            m = jnp.max(jnp.maximum(s0, s), axis=-1, keepdims=True)
                        else:
                            m = jnp.max(jnp.maximum(fold(s0, jnp.maximum), fold(s, jnp.maximum)), axis=-1, keepdims=True)
                        p0 = jnp.exp2(s0 - m); p1 = jnp.exp2(s - m)
                        if sm in "ac":
                            st["l", h] = jnp.sum(p0 + p1, axis=-1, keepdims=True)
                        else:
                            st["l", h] = jnp.sum(fold(p0, jnp.add) + fold(p1, jnp.add), axis=-1, keepdims=True)
                        st["p", h, 0] = p0.astype(bf16); st["p", h, 1] = p1.astype(bf16)
                return (lambda: ldw(slot * KV + k * 512), lambda: q_s[h],
                        lambda a, w: lax.dot_general(a, w, NT, preferred_element_type=f32), fin)
            def P(k):
                h, u = divmod(k, 2)
                def fin(o):
                    if u == 0:
                        st["o", h] = o
                    else:
                        l = st["l", h]
                        r = pl.reciprocal(l, approx=True)
                        if newton: r = r * (2.0 - l * r)
                        st["o", h] = ((o + st["o", h]) * r).astype(bf16)
                return lambda: ldw(slot * KV + G * Sk + k * 512), lambda: st["p", h, u], nn, fin
            def O(k):
                kk, n = divmod(k, 4)
                def fin(r):
                    if kk == 0:
                        acc[b, n] = r + jnp.where((ph & 3) == 0, 0.0, acc[b, n])
                    else:
                        r = r + acc[b, n]
                        acc[b, n] = r
                        out_s[b, :, pl.ds(pl.multiple_of((i >> 6) * D + n * 128, 128), 128)] = r.astype(bf16)
                return (lambda: wo_s[ph, pl.ds(kk * 512, 512), pl.ds(n * 128, 128)],
                        lambda: jnp.concatenate([st["o", h] if ("o", h) in st else pltpu.bitcast(buf.bitcast(u32)[pl.ds((NG * KV + h * Sq) // 2, Sq // 2), :], bf16)
                                                 for h in range(kk * 4, kk * 4 + 4)], axis=1), nn, fin)
            stages = [dict(Q=Q, S=S, P=P, O=O)[c](names[:t].count(c)) for t, c in enumerate(names)]
            w = stages[0][0]()
            res = None
            for t, (_, lhs, mm, fin) in enumerate(stages):
                issue(t)
                if t:
                    stages[t - 1][3](res)
                for h in range(G):
                    if odl and (olast or h % 4 != 3) and t == [q for q, c in enumerate(names) if c == "P"][2 * h + 1] + (olast if h % 4 == 3 else odl):
                        buf[pl.ds(NG * KV + h * Sq, Sq), :] = st.pop(("o", h))
                a = lhs()
                wn = stages[t + 1][0]() if t + 1 < NP else None
                res = mm(a, w)
                w = wn
            stages[-1][3](res)
            arrive(i + 1, slot1)
            return slot1
        lax.fori_loop(0, N, body, jnp.int32(0))
        for u in range(10):
            out_piece(B - 1, u).start(priority=u % 2)
        if ballast:
            @pl.loop(0, (N - 2 - 80) * 4)
            def _(t):
                wq_piece(awq, 0, t).wait()
        if scope:
            with jax.named_scope('outwait'):
                full_wait(out_s, WS)
        else:
            full_wait(out_s, WS)

    def kernel_v14(*a):
        a = [t.reshape(B * H * Sk, Dh) if t.ndim == 4 else t for t in a]
        return pl.pallas_call(
            kern,
            in_specs=([pl.BlockSpec(memory_space=pltpu.SMEM)] if table else []) + [pl.BlockSpec(memory_space=pl.ANY)] * 10,
            out_specs=pl.BlockSpec(memory_space=pl.ANY),
            out_shape=jax.ShapeDtypeStruct((B, Sq, 2 * D), bf16),
            scratch_shapes=[
                pltpu.VMEM((NG * KV + G * Sq, Dh), bf16),
                pltpu.VMEM((2, D, H * Dh + qpad), bf16), pltpu.VMEM((8, G * Dh, D), bf16),
                pltpu.VMEM((2 * B, Sq, D), bf16),
                pltpu.VMEM((G, Sq, Dh), bf16),
                pltpu.VMEM((B, 4, Sq, 128), f32), pltpu.VMEM((B, Sq, 2 * D), bf16),
                pltpu.SemaphoreType.DMA((NG + 9,))],
            compiler_params=pltpu.CompilerParams(vmem_limit_bytes=120 * 2**20, disable_bounds_checks=True, disable_semaphore_checks=nosemchk, flags=flags),
        )(*a)
    kernel_v14.hoff = hoff
    return kernel_v14


@jax.jit
def pallas_concat_heads__mha_block_cached__gqa_block_cached__near_ridge_kernel(
        A_x, A_k_cache, A_v_cache, A_wq, A_wo, B_x, B_k_cache, B_v_cache, B_wq, B_wo):
    return make()(A_x, A_k_cache, A_v_cache, A_wq, A_wo, B_x, B_k_cache, B_v_cache, B_wq, B_wo)
```

```python
import math

import jax
import jax.numpy as jnp
from jax import lax
from jax.experimental import pallas as pl
from jax.experimental.pallas import tpu as pltpu

B, SQ, D, H, SK, DH = 16, 160, 512, 32, 1024, 128
Q_SCALE = DH**-0.5 * math.log2(math.e)

G = 8
GROUPS = H // G
HALF = B * GROUPS
STEPS = 2 * HALF
SLOTS = 3
SLOT_ROWS = 2 * G * SK
O_BASE = SLOTS * SLOT_ROWS
CHUNK = 128
TILES = 4 * 128
X_ROWS = SQ // GROUPS
X_AHEAD = GROUPS + 1
W_PIECES = 128
W_EARLY = 8
OUT_ROWS = 16
SEM_WQ, SEM_WO, SEM_X, SEM_OUT = SLOTS, SLOTS + 2, SLOTS + 4, SLOTS + 5

STAGES = "QSSQPP" "SSQPP" "SSQPP" "SSQSPP" "SOQPP" "SSOPP" "SSQPO" "SSOPPPQ" "OOOO"


def _kv_copies():
    heads = (0, 5, 2, 3, 4, 1, 6, 7)
    chunks = (1, 0, 7, 3, 4, 5, 6, 2)
    priority = (0, 1, 1, 0, 1, 1, 0, 1)
    return [
        (a, heads[e], chunks[(r + 3 * (1 - priority[e])) % len(chunks)], priority[e])
        for a in range(2)
        for r in range(len(chunks))
        for e in range(G)
    ]


def _kv_schedule():
    copies = _kv_copies()
    half = len(copies) // 2
    plan, c = [], half
    for t in range(len(STAGES)):
        n = (3, 3, 2)[t % 3]
        plan.append((1 + c // len(copies), copies[c % len(copies):][:n]))
        c += n
    assert c == half + len(copies)
    return plan


def _out_schedule():
    n = (B - 1) * SQ // OUT_ROWS
    pieces = [w for c in range(16) for w in range(c, n, 16)]
    sites = [(STEPS - 2, t) for t in range(len(STAGES) - 12, len(STAGES))]
    sites += [(STEPS - 1, t) for t in range(36)]
    plan = {}
    for k, w in enumerate(pieces):
        site = sites[k * len(sites) // n]
        urgent = site[0] == STEPS - 1 and k % 3 == 2
        plan.setdefault(site, []).append((w, 0 if urgent else 1))
    return plan


def _span(start, size):
    if not isinstance(start, int):
        start = pl.multiple_of(start, math.gcd(size, 128))
    return pl.ds(start, size)


def _dot(a, b):
    return jnp.dot(a, b, preferred_element_type=jnp.float32)


def _dot_nt(a, b):
    return lax.dot_general(
        a, b, (((1,), (1,)), ((), ())), preferred_element_type=jnp.float32
    )


def _fold_max(s):
    return jnp.maximum(
        jnp.maximum(s[:, :128], s[:, 128:256]), jnp.maximum(s[:, 256:384], s[:, 384:])
    )


def _kernel(a_x, a_k, a_v, a_wq, a_wo, b_x, b_k, b_v, b_wq, b_wo, out_hbm,
            buf, wq_s, wo_s, x_s, q_s, acc, out_s, sem):
    kv_plan, out_plan = _kv_schedule(), _out_schedule()

    def batch(i):
        return i >> 2

    def head(i, j):
        return (i & (GROUPS - 1)) + GROUPS * j

    def block(i):
        return i >> 6

    def kv_copy(caches, i, slot, a, j, c):
        src = ((batch(i) & (B - 1)) * H + head(i, 0)) * SK + (GROUPS * j * SK + c * CHUNK)
        dst = slot * SLOT_ROWS + ((a * G + j) * SK + c * CHUNK)
        return pltpu.make_async_copy(
            caches[a].at[_span(src, CHUNK)], buf.at[_span(dst, CHUNK)], sem.at[slot]
        )

    def kv_start(caches, i, slot, copies):
        for a, j, c, priority in copies:
            kv_copy(caches, i, slot, a, j, c).start(priority=priority)

    def kv_wait(slot):
        rows = buf.at[_span(slot * SLOT_ROWS, SLOT_ROWS)]
        pltpu.make_async_copy(rows, rows, sem.at[slot]).wait()

    def wq_copy(wq, blk, t):
        t = (t * 17) & (W_PIECES - 1)
        r, c = _span((t >> 1) * 8, 8), _span((t & 1) * 2048, 2048)
        return pltpu.make_async_copy(wq.at[r, c], wq_s.at[blk, r, c], sem.at[SEM_WQ + blk])

    def wo_copy(wo, blk, t):
        r = _span(((t * 17) & (W_PIECES - 1)) * 32, 32)
        return pltpu.make_async_copy(wo.at[r], wo_s.at[blk, r], sem.at[SEM_WO + blk])

    def weights_wait(wq, wo, blk):
        pltpu.make_async_copy(
            wq, wq_s.at[blk, :, pl.ds(0, H * DH)], sem.at[SEM_WQ + blk]
        ).wait()
        pltpu.make_async_copy(wo, wo_s.at[blk], sem.at[SEM_WO + blk]).wait()

    def out_copy(w):
        r = pl.ds(w * OUT_ROWS, OUT_ROWS)
        return pltpu.make_async_copy(out_s.at[r], out_hbm.at[r], sem.at[SEM_OUT])

    def x_tile(i):
        return x_s[_span(batch(i) * SQ, SQ), :]

    def wq_tile(i, j):
        return wq_s[block(i), :, _span(head(i, j) * DH, DH)]

    first_x = pl.ds(0, X_AHEAD * X_ROWS)
    x_head = pltpu.make_async_copy(a_x.at[first_x], x_s.at[first_x], sem.at[SEM_X])
    x_head.start(priority=1)

    @pl.loop(0, W_PIECES // 2)
    def _(n):
        for a in range(2):
            wq_copy(a_wq, 0, 2 * n + a).start(priority=1)
            wo_copy(a_wo, 0, 2 * n + a).start(priority=1)
            kv_copy((a_k, a_v), 0, 0, a, n & (G - 1), n >> 3).start(priority=0)

    @pl.loop(0, W_EARLY)
    def _(t):
        wq_copy(b_wq, 1, t).start(priority=1)
        wo_copy(b_wo, 1, t).start(priority=0)

    kv_start((a_k, a_v), 1, 1, [e for e in _kv_copies() if e[0] == 0])
    acc[...] = jnp.zeros_like(acc)
    x_head.wait()
    weights_wait(a_wq, a_wo, 0)
    q_s[0] = (_dot(x_tile(0), wq_tile(0, 0)) * Q_SCALE).astype(q_s.dtype)
    kv_wait(0)

    def step(i, slot):
        slots = {
            1: jnp.where(slot == SLOTS - 1, 0, slot + 1),
            2: jnp.where(slot == 0, SLOTS - 1, slot - 1),
        }

        def per_block(e, for_a, for_b):
            pl.when(e < HALF)(for_a)
            pl.when(jnp.logical_and(e >= HALF, e < STEPS))(for_b)

        def x_copy(x):
            e = i + X_AHEAD
            return pltpu.make_async_copy(
                x.at[_span((e & (HALF - 1)) * X_ROWS, X_ROWS)],
                x_s.at[_span(e * X_ROWS, X_ROWS)],
                sem.at[SEM_X],
            )

        def start_copies(t, kind, k):
            if kind in "QO":
                piece = W_EARLY + 2 * i + k // 4
                turn = (k + 2) & 3 if kind == "Q" else k & 3

                @pl.when(jnp.logical_and((i & 3) == turn, piece < W_PIECES))
                def _():
                    if kind == "Q":
                        wq_copy(b_wq, 1, piece).start(priority=1)
                    else:
                        wo_copy(b_wo, 1, piece).start(priority=1)

            ahead, copies = kv_plan[t]
            per_block(
                i + ahead,
                lambda: kv_start((a_k, a_v), i + ahead, slots[ahead], copies),
                lambda: kv_start((b_k, b_v), i + ahead, slots[ahead], copies),
            )
            if t == 5:
                per_block(
                    i + X_AHEAD,
                    lambda: x_copy(a_x).start(priority=1),
                    lambda: x_copy(b_x).start(priority=1),
                )
            for last in (STEPS - 2, STEPS - 1):
                if (last, t) in out_plan:

                    @pl.when(i == last)
                    def _():
                        for w, priority in out_plan[last, t]:
                            out_copy(w).start(priority=priority)

        scores, probs, sums, outs = {}, {}, {}, {}

        def q_stage(k):
            it, j = (i, k + 1) if k < G - 1 else (jnp.minimum(i + 1, STEPS - 1), 0)

            def finish(q):
                q_s[j] = (q * Q_SCALE).astype(q_s.dtype)

            return lambda: wq_tile(it, j), lambda: x_tile(it), _dot, finish

        def s_stage(k):
            j, u = divmod(k, 2)

            def finish(s):
                scores[j, u] = s
                if u == 1:
                    s0, s1 = scores[j, 0], s
                    m = jnp.maximum(_fold_max(s0), _fold_max(s1))
                    m = jnp.max(m, axis=-1, keepdims=True)
                    p0, p1 = jnp.exp2(s0 - m), jnp.exp2(s1 - m)
                    sums[j] = jnp.sum(p0 + p1, axis=-1, keepdims=True)
                    probs[j, 0], probs[j, 1] = p0.astype(buf.dtype), p1.astype(buf.dtype)

            keys = lambda: buf[_span(slot * SLOT_ROWS + k * TILES, TILES), :]
            return keys, lambda: q_s[j], _dot_nt, finish

        def p_stage(k):
            j, u = divmod(k, 2)

            def finish(o):
                if u == 0:
                    outs[j] = o
                else:
                    r = pl.reciprocal(sums[j], approx=True)
                    r = r * (2.0 - sums[j] * r)
                    outs[j] = ((o + outs[j]) * r).astype(buf.dtype)

            values = lambda: buf[_span(slot * SLOT_ROWS + (G * SK + k * TILES), TILES), :]
            return values, lambda: probs[j, u], _dot, finish

        def o_stage(k):
            part, n = divmod(k, 4)
            js = range(4 * part, 4 * part + 4)

            def weights():
                cols = pl.ds(n * 128, 128)
                return jnp.concatenate(
                    [wo_s[block(i), _span(head(i, j) * DH, DH), cols] for j in js], axis=0
                )

            def heads():
                return jnp.concatenate(
                    [outs[j] if j in outs else buf[pl.ds(O_BASE + j * SQ, SQ), :] for j in js],
                    axis=1,
                )

            def finish(r):
                if part == 0:
                    acc[n] = r + jnp.where((i & (GROUPS - 1)) == 0, 0.0, acc[n])
                else:
                    r = r + acc[n]
                    acc[n] = r
                    rows = _span((batch(i) & (B - 1)) * SQ, SQ)
                    out_s[rows, _span(block(i) * D + n * 128, 128)] = r.astype(out_s.dtype)

            return weights, heads, _dot, finish

        build = {"Q": q_stage, "S": s_stage, "P": p_stage, "O": o_stage}
        index = [STAGES[:t].count(kind) for t, kind in enumerate(STAGES)]
        stages = [build[kind](k) for kind, k in zip(STAGES, index)]
        park = {
            t + 2: k // 2
            for t, (kind, k) in enumerate(zip(STAGES, index))
            if kind == "P" and k % 2 == 1 and k // 2 in (1, 2, 5)
        }

        stationary, result = stages[0][0](), None
        for t, (_, moving, matmul, _) in enumerate(stages):
            start_copies(t, STAGES[t], index[t])
            if t > 0:
                stages[t - 1][3](result)
            if t in park:
                buf[pl.ds(O_BASE + park[t] * SQ, SQ), :] = outs.pop(park[t])
            lhs = moving()
            following = stages[t + 1][0]() if t + 1 < len(stages) else None
            result = matmul(lhs, stationary)
            stationary = following
        stages[-1][3](result)

        pl.when(i + 1 < STEPS)(lambda: kv_wait(slots[1]))
        pl.when(i + X_AHEAD < STEPS)(lambda: x_copy(a_x).wait())
        pl.when(i == HALF - 2)(lambda: weights_wait(b_wq, b_wo, 1))
        return slots[1]

    lax.fori_loop(0, STEPS, step, jnp.int32(0))

    for w in range((B - 1) * SQ // OUT_ROWS, B * SQ // OUT_ROWS):
        out_copy(w).start(priority=1 - w % 2)
    pltpu.make_async_copy(out_s, out_hbm, sem.at[SEM_OUT]).wait()


@jax.jit
def pallas_concat_heads__mha_block_cached__gqa_block_cached__near_ridge_kernel(
    A_x: jax.Array,
    A_k_cache: jax.Array,
    A_v_cache: jax.Array,
    A_wq: jax.Array,
    A_wo: jax.Array,
    B_x: jax.Array,
    B_k_cache: jax.Array,
    B_v_cache: jax.Array,
    B_wq: jax.Array,
    B_wo: jax.Array,
):
    assert A_x.shape == B_x.shape == (B, SQ, D)
    assert A_k_cache.shape == A_v_cache.shape == (B, H, SK, DH)
    assert B_k_cache.shape == B_v_cache.shape == (B, H, SK, DH)
    dtype = A_x.dtype
    operands = [A_x, A_k_cache, A_v_cache, A_wq, A_wo, B_x, B_k_cache, B_v_cache, B_wq, B_wo]
    out = pl.pallas_call(
        _kernel,
        in_specs=[pl.BlockSpec(memory_space=pl.ANY)] * len(operands),
        out_specs=pl.BlockSpec(memory_space=pl.ANY),
        out_shape=jax.ShapeDtypeStruct((B * SQ, 2 * D), dtype),
        scratch_shapes=[
            pltpu.VMEM((O_BASE + G * SQ, DH), dtype),
            pltpu.VMEM((2, D, H * DH + 128), dtype),
            pltpu.VMEM((2, H * DH, D), dtype),
            pltpu.VMEM((2 * B * SQ, D), dtype),
            pltpu.VMEM((G, SQ, DH), dtype),
            pltpu.VMEM((D // 128, SQ, 128), jnp.float32),
            pltpu.VMEM((B * SQ, 2 * D), dtype),
            pltpu.SemaphoreType.DMA((SEM_OUT + 1,)),
        ],
        compiler_params=pltpu.CompilerParams(
            vmem_limit_bytes=64 * 2**20,
            disable_bounds_checks=True,
            disable_semaphore_checks=True,
        ),
    )(*[a.reshape(-1, a.shape[-1]) for a in operands])
    return out.reshape(B, SQ, 2 * D)
```
